```python
import os as _os
_os.environ.setdefault("JAX_PLATFORMS", "cpu")
import jax
import jax.numpy as jnp

def _softmax(x, axis=-1):
    return jax.nn.softmax(x, axis=axis)
def _gelu(x):
    return jax.nn.gelu(x, approximate=True)
def _silu(x):
    return jax.nn.silu(x)
def _sigmoid(x):
    return jax.nn.sigmoid(x)
def _layernorm(x, axis=-1, eps=1e-5):
    m = jnp.mean(x, axis=axis, keepdims=True)
    v = jnp.var(x, axis=axis, keepdims=True)
    return (x - m) / jnp.sqrt(v + eps)
def _scatter_add(tgt, idx, src, axis=0):
    return tgt.at[idx].add(src)
def _segment_sum(src, seg, n):
    return jax.ops.segment_sum(src, seg, n)
class _Rng:
    def __init__(self, key):
        self._k = key
    def _next(self):
        self._k, sub = jax.random.split(self._k)
        return sub
    def normal(self, shape):
        return jax.random.normal(self._next(), shape, dtype=jnp.bfloat16)
    def randint(self, lo, hi, shape):
        return jax.random.randint(self._next(), shape, lo, hi, dtype=jnp.int32)
    def uniform(self, shape, lo=0.0, hi=1.0):
        return jax.random.uniform(self._next(), shape, jnp.bfloat16, lo, hi)
    def permutation(self, n):
        return jax.random.permutation(self._next(), n)


kernel_name = 'standalone__gqa_softmax__near_ridge'

def setup_inputs():
    _rng = _Rng(jax.random.key(int.from_bytes(__import__("os").urandom(4), "little")))
    _w = (lambda a: (lambda t: t.astype(jnp.bfloat16) if jnp.issubdtype(t.dtype, jnp.floating) else t)(jnp.asarray(a)))
    B, Hq, Hkv, Sq, Sk, D = 8, 16, 8, 512, 512, 256
    return {
        "q": _w((lambda *s: _rng.normal(s) * 0.4)(B, Hq, Sq, D)),
        "k": _w((lambda *s: _rng.normal(s) * 0.4)(B, Hkv, Sk, D)),
        "v": _w((lambda *s: _rng.normal(s) * 0.05)(B, Hkv, Sk, D)),
    }

def reference(q, k, v):
    B, Hq, Sq, D = q.shape
    Hkv = k.shape[1]
    rep = Hq // Hkv
    k = jnp.repeat(k, rep, axis=1)
    v = jnp.repeat(v, rep, axis=1)
    scale = D ** -0.5
    scores = jnp.einsum("bhqd,bhkd->bhqk", q, k) * scale
    p = _softmax(scores, axis=-1)
    return jnp.einsum("bhqk,bhkd->bhqd", p, v)
```

```python
import functools

import jax
import jax.numpy as jnp
import jax.experimental.pallas as pl
import jax.experimental.pallas.tpu as pltpu


def _attn_kernel(q_ref, k_ref, v_ref, o_ref, *, tq, scale):
    k = k_ref[...]
    v = v_ref[...]
    n = q_ref.shape[0] // tq
    for c in range(n):
        q = q_ref[pl.ds(c * tq, tq), :]
        s = jax.lax.dot_general(q, k, (((1,), (1,)), ((), ())),
                                preferred_element_type=jnp.float32)
        m = jnp.max(s, axis=-1, keepdims=True)
        p = jnp.exp((s - m) * scale)
        l = jnp.sum(p, axis=-1, keepdims=True)
        o = jnp.dot(p.astype(jnp.bfloat16), v, preferred_element_type=jnp.float32)
        o_ref[pl.ds(c * tq, tq), :] = (o * (1.0 / l)).astype(o_ref.dtype)


@jax.jit
def pallas_standalone__gqa_softmax__near_ridge_kernel(q, k, v):
    B, Hq, Sq, D = q.shape
    Hkv, Sk = k.shape[1], k.shape[2]
    rep = Hq // Hkv
    scale = float(D) ** -0.5
    qr = q.reshape(B * Hkv, rep * Sq, D)
    kr = k.reshape(B * Hkv, Sk, D)
    vr = v.reshape(B * Hkv, Sk, D)
    out = pl.pallas_call(
        functools.partial(_attn_kernel, tq=256, scale=scale),
        grid=(B * Hkv,),
        in_specs=[
            pl.BlockSpec((None, rep * Sq, D), lambda i: (i, 0, 0)),
            pl.BlockSpec((None, Sk, D), lambda i: (i, 0, 0)),
            pl.BlockSpec((None, Sk, D), lambda i: (i, 0, 0)),
        ],
        out_specs=pl.BlockSpec((None, rep * Sq, D), lambda i: (i, 0, 0)),
        out_shape=jax.ShapeDtypeStruct((B * Hkv, rep * Sq, D), q.dtype),
        compiler_params=pltpu.CompilerParams(
            dimension_semantics=("parallel",),
            vmem_limit_bytes=64 * 1024 * 1024,
        ),
    )(qr, kr, vr)
    return out.reshape(B, Hq, Sq, D)
```

```python
import functools

import jax
import jax.numpy as jnp
import jax.experimental.pallas as pl
import jax.experimental.pallas.tpu as pltpu

_LOG2E = 1.4426950408889634
_TQ = 128
_DEPTH = 2
_NSEM = 2


def _make_items(ngroups, rows, first_chunks=()):
    items, off = [], 0
    for c in first_chunks:
        items.append((0, off, c))
        off += c
    while off < rows:
        items.append((0, off, _TQ))
        off += _TQ
    for g in range(1, ngroups):
        for c in range(rows // _TQ):
            items.append((g, c * _TQ, _TQ))
    return items


def _block_ops(n):
    ops, nq, npv = [], 0, 0
    while npv < n:
        if nq < n and nq - npv <= _DEPTH:
            ops.append(("q", nq))
            nq += 1
        else:
            ops += [("s", npv), ("p", npv)]
            npv += 1
    return ops


def _ramp_ops(items, ramp_sizes, nfirst):
    n = len(items)
    ops = [("f", 0)]
    ops += [("q", j) for j in range(nfirst)]
    ops += [("s", j) for j in range(nfirst - 1)]
    ops.append(("f", 1))
    nq, ns, npv, g = nfirst, nfirst - 1, 0, 2
    firsts, acc = [], 1
    for sz in ramp_sizes:
        firsts.append(acc)
        acc += sz
    bounds = [j for j, it in enumerate(items) if it[0] in firsts and it[1] == 0]
    after_fence = True
    while npv < n:
        want_q = nq < n and nq - npv <= _DEPTH
        if after_fence and npv < ns:
            want_q = False
        after_fence = False
        if want_q and nq in bounds:
            while ns < nq - 1:
                ops.append(("s", ns))
                ns += 1
            ops.append(("f", g))
            g += 1
            bounds.remove(nq)
            after_fence = True
        elif want_q:
            ops.append(("q", nq))
            nq += 1
        else:
            if ns <= npv:
                ops.append(("s", ns))
                ns += 1
            ops.append(("p", npv))
            npv += 1
    return ops


def _attn_kernel(q_hbm, k_hbm, v_hbm, o_hbm, qb, kb, vb, ob, sem_in, sem_out, *,
                 scale, ramp_sizes, nfirst, blk, nblk, ramp_out_step):
    rows = qb.shape[1]
    ramp = 1 + sum(ramp_sizes)
    ramp_items = _make_items(ramp, rows)
    main_items = _make_items(blk, rows, (_TQ, _TQ, 2 * _TQ))
    first_rows = nfirst * _TQ

    def group_copies(g0, n, sem):
        sl = pl.ds(g0, n)
        return [pltpu.make_async_copy(k_hbm.at[sl], kb.at[sl], sem),
                pltpu.make_async_copy(q_hbm.at[sl], qb.at[sl], sem),
                pltpu.make_async_copy(v_hbm.at[sl], vb.at[sl], sem)]

    def first_copies(sem):
        sl = pl.ds(0, first_rows)
        return [pltpu.make_async_copy(k_hbm.at[0], kb.at[0], sem),
                pltpu.make_async_copy(q_hbm.at[0, sl], qb.at[0, sl], sem)]

    def second_copies(sem):
        sl = pl.ds(first_rows, rows - first_rows)
        return [pltpu.make_async_copy(v_hbm.at[0], vb.at[0], sem),
                pltpu.make_async_copy(q_hbm.at[0, sl], qb.at[0, sl], sem)]

    dma_groups = [first_copies, second_copies]
    g0 = 1
    for sz in ramp_sizes:
        dma_groups.append(functools.partial(group_copies, g0, sz))
        g0 += sz
    n_ramp_dma = len(dma_groups)
    for t in range(nblk):
        dma_groups.append(functools.partial(group_copies, ramp + t * blk, blk))

    def start_group(g):
        if g < len(dma_groups):
            for c in dma_groups[g](sem_in.at[g % _NSEM]):
                c.start()

    def out_copy(g, r0, n):
        sl = pl.ds(r0, n)
        return pltpu.make_async_copy(ob.at[g, sl], o_hbm.at[g, sl], sem_out.at[0])

    def emit(ops, items, base, exp2_items, fence, write_out):
        scores, probs = {}, {}
        last_group = items[-1][0]
        for op, j in ops:
            if op == "f":
                fence(j)
                continue
            gl, r0, n = items[j]
            g = base + gl
            if op == "q":
                scores[j] = jax.lax.dot_general(
                    qb[g, pl.ds(r0, n), :], kb[g], (((1,), (1,)), ((), ())),
                    preferred_element_type=jnp.float32)
            elif op == "s":
                s = scores.pop(j)
                m = jnp.max(s, axis=-1, keepdims=True)
                if j in exp2_items:
                    p = jnp.exp2((s - m) * (scale * _LOG2E))
                else:
                    p = jnp.exp((s - m) * scale)
                l = jnp.sum(p, axis=-1, keepdims=True)
                r = pl.reciprocal(l, approx=True)
                r = r * (2.0 - l * r)
                probs[j] = (p * r).astype(vb.dtype)
            else:
                o = jnp.dot(probs.pop(j), vb[g], preferred_element_type=jnp.float32)
                ob[g, pl.ds(r0, n), :] = o.astype(ob.dtype)
                if write_out:
                    if gl == last_group:
                        out_copy(g, r0, n).start()
                    elif r0 + n == rows:
                        out_copy(g, 0, rows).start()

    for g in range(_NSEM):
        start_group(g)

    def ramp_fence(g):
        for c in dma_groups[g](sem_in.at[g % _NSEM]):
            c.wait()
        start_group(g + _NSEM)

    emit(_ramp_ops(ramp_items, ramp_sizes, nfirst), ramp_items, 0, (), ramp_fence, False)

    main_ops = _block_ops(len(main_items))

    def body(t, carry):
        base = ramp + t * blk
        sem = sem_in.at[(n_ramp_dma + t) % _NSEM]
        for c in group_copies(base, blk, sem):
            c.wait()

        @pl.when(t + _NSEM < nblk)
        def _():
            for c in group_copies(base + _NSEM * blk, blk, sem):
                c.start()

        @pl.when(t == ramp_out_step)
        def _():
            sl = pl.ds(0, ramp)
            pltpu.make_async_copy(ob.at[sl], o_hbm.at[sl], sem_out.at[0]).start()

        emit(main_ops, main_items, base, (0, 1, 2), None, True)
        return carry

    jax.lax.fori_loop(0, nblk, body, 0)

    pltpu.make_async_copy(ob, o_hbm, sem_out.at[0]).wait()


@jax.jit
def pallas_standalone__gqa_softmax__near_ridge_kernel(q, k, v):
    B, Hq, Sq, D = q.shape
    Hkv, Sk = k.shape[1], k.shape[2]
    rep = Hq // Hkv
    G, rows = B * Hkv, rep * Sq
    ramp_sizes, blk, nblk = (1, 2, 4), 8, 7
    assert 1 + sum(ramp_sizes) + blk * nblk == G and rows % (4 * _TQ) == 0

    out = pl.pallas_call(
        functools.partial(_attn_kernel, scale=float(D) ** -0.5, ramp_sizes=ramp_sizes,
                          nfirst=4, blk=blk, nblk=nblk, ramp_out_step=3),
        in_specs=[pl.BlockSpec(memory_space=pl.ANY)] * 3,
        out_specs=pl.BlockSpec(memory_space=pl.ANY),
        out_shape=jax.ShapeDtypeStruct((G, rows, D), q.dtype),
        scratch_shapes=[
            pltpu.VMEM((G, rows, D), q.dtype),
            pltpu.VMEM((G, Sk, D), k.dtype),
            pltpu.VMEM((G, Sk, D), v.dtype),
            pltpu.VMEM((G, rows, D), q.dtype),
            pltpu.SemaphoreType.DMA((_NSEM,)),
            pltpu.SemaphoreType.DMA((1,)),
        ],
        compiler_params=pltpu.CompilerParams(
            vmem_limit_bytes=120 * 1024 * 1024,
            disable_bounds_checks=True,
        ),
    )(q.reshape(G, rows, D), k.reshape(G, Sk, D), v.reshape(G, Sk, D))
    return out.reshape(B, Hq, Sq, D)
```

```python
import functools

import jax
import jax.numpy as jnp
import jax.experimental.pallas as pl
import jax.experimental.pallas.tpu as pltpu

_LOG2E = 1.4426950408889634
_TQ = 128
_DEPTH = 2
_NSEM = 2
_KT = 256
_LAST_SPLIT = 4
_NT = (((1,), (1,)), ((), ()))


def _make_items(ngroups, rows, first_chunks=()):
    items, off = [], 0
    for c in first_chunks:
        items.append((0, off, c))
        off += c
    while off < rows:
        items.append((0, off, _TQ))
        off += _TQ
    for g in range(1, ngroups):
        for c in range(rows // _TQ):
            items.append((g, c * _TQ, _TQ))
    return items


def _block_ops(n):
    ops, nq, npv = [], 0, 0
    while npv < n:
        if nq < n and nq - npv <= _DEPTH:
            ops.append(("q", nq))
            nq += 1
        else:
            ops += [("s", npv), ("p", npv)]
            npv += 1
    return ops


def _ramp_ops(items, ramp_sizes, nfirst):
    n = len(items)
    firsts, acc = [], 1
    for sz in ramp_sizes:
        firsts.append(acc)
        acc += sz
    bounds = [j for j, it in enumerate(items) if it[0] in firsts and it[1] == 0]
    mxu = [("f", 0)] + [("q", j) for j in range(nfirst)] + [("f", 1)]
    nq, npv, g = nfirst, 0, 2
    while npv < n:
        if nq < n and nq - npv <= _DEPTH:
            mxu.append(("q", nq))
            nq += 1
        else:
            if nq in bounds and nq - npv == _DEPTH + 1:
                mxu.append(("f", g))
                g += 1
                bounds.remove(nq)
            mxu.append(("p", npv))
            npv += 1
    ops, ns, nq = [], 0, 0
    for op, j in mxu:
        upto = {"f": nq - 1, "p": j + 1, "q": 0}[op]
        while ns < upto:
            ops.append(("s", ns))
            ns += 1
        nq += op == "q"
        ops.append((op, j))
    return ops


def _attn_kernel(q_hbm, k_hbm, v_hbm, o_hbm, qb, kb, vb, ob, kf, kt,
                 sem_in, sem_out, one_ref, *,
                 scale, ramp_sizes, nfirst, blk, nblk, ramp_out_step):
    ngroups, rows = qb.shape[0], qb.shape[1]
    ramp = 1 + sum(ramp_sizes)
    ramp_items = _make_items(ramp, rows)
    main_items = _make_items(blk, rows, (_TQ, _TQ, 2 * _TQ))
    first_rows = nfirst * _TQ

    def group_copies(g0, n, kf_slot, sem):
        sl = pl.ds(g0, n)
        cps = [pltpu.make_async_copy(k_hbm.at[sl], kb.at[sl], sem),
               pltpu.make_async_copy(q_hbm.at[sl], qb.at[sl], sem),
               pltpu.make_async_copy(v_hbm.at[sl], vb.at[sl], sem)]
        if kf_slot is not None:
            nxt = jnp.minimum(g0 + n, ngroups - 1)
            cps.append(pltpu.make_async_copy(
                k_hbm.at[nxt, pl.ds(0, _KT)], kf.at[kf_slot], sem))
        return cps

    def first_copies(sem):
        sl = pl.ds(0, first_rows)
        return [pltpu.make_async_copy(k_hbm.at[0], kb.at[0], sem),
                pltpu.make_async_copy(q_hbm.at[0, sl], qb.at[0, sl], sem)]

    def second_copies(sem):
        sl = pl.ds(first_rows, rows - first_rows)
        return [pltpu.make_async_copy(v_hbm.at[0], vb.at[0], sem),
                pltpu.make_async_copy(q_hbm.at[0, sl], qb.at[0, sl], sem)]

    dma_groups = [first_copies, second_copies]
    g0 = 1
    for i, sz in enumerate(ramp_sizes):
        slot = 0 if i == len(ramp_sizes) - 1 else None
        dma_groups.append(functools.partial(group_copies, g0, sz, slot))
        g0 += sz
    n_ramp_dma = len(dma_groups)
    for t in range(nblk):
        dma_groups.append(functools.partial(group_copies, ramp + t * blk, blk, t + 1))

    def start_group(g):
        for c in dma_groups[g](sem_in.at[g % _NSEM]):
            c.start()

    def out_copy(g, r0, n):
        sl = pl.ds(r0, n)
        return pltpu.make_async_copy(ob.at[g, sl], o_hbm.at[g, sl], sem_out.at[0])

    def emit(ops, items, base, kf_slot, exp2_items, fence, main):
        scores, probs = {}, {}
        last_group = items[-1][0]
        for idx, (op, j) in enumerate(ops):
            if idx == len(ops) - 20:
                kt[...] = kf[kf_slot].T
            if op == "f":
                fence(j)
                continue
            gl, r0, n = items[j]
            g = base + gl
            if op == "q":
                qv = qb[g, pl.ds(r0, n), :]
                if main and j == 0:
                    s0 = jnp.dot(qv, kt[...], preferred_element_type=jnp.float32)
                    s1 = jax.lax.dot_general(
                        qv, kb[g, pl.ds(_KT, kb.shape[1] - _KT), :], _NT,
                        preferred_element_type=jnp.float32)
                    scores[j] = jnp.concatenate([s0, s1], axis=1)
                else:
                    scores[j] = jax.lax.dot_general(
                        qv, kb[g], _NT, preferred_element_type=jnp.float32)
            elif op == "s":
                s = scores.pop(j)
                m = jnp.max(s, axis=-1, keepdims=True)
                if j in exp2_items:
                    p = jnp.exp2((s - m) * (scale * _LOG2E))
                else:
                    p = jnp.exp((s - m) * scale)
                l = jnp.sum(p, axis=-1, keepdims=True)
                r = pl.reciprocal(l, approx=True)
                r = r * (2.0 - l * r)
                probs[j] = (p * r).astype(vb.dtype)
            else:
                o = jnp.dot(probs.pop(j), vb[g],
                            preferred_element_type=jnp.float32).astype(ob.dtype)
                if main and j == len(items) - 1:
                    per = n // _LAST_SPLIT
                    for u in range(_LAST_SPLIT):
                        ob[g, pl.ds(r0 + u * per, per), :] = o[u * per:(u + 1) * per]
                        out_copy(g, r0 + u * per, per).start()
                    continue
                ob[g, pl.ds(r0, n), :] = o
                if main and gl == last_group:
                    out_copy(g, r0, n).start()
                elif main and r0 + n == rows:
                    out_copy(g, 0, rows).start()

    def ramp_fence(g):
        for c in dma_groups[g](sem_in.at[g % _NSEM]):
            c.wait()
        start_group(g + _NSEM)

    ramp_ops = _ramp_ops(ramp_items, ramp_sizes, nfirst)
    main_ops = _block_ops(len(main_items))

    def main_block(t, carry):
        base = ramp + t * blk
        sem = sem_in.at[(n_ramp_dma + t) % _NSEM]
        for c in group_copies(base, blk, t + 1, sem):
            c.wait()

        @pl.when(t + _NSEM < nblk)
        def _():
            for c in group_copies(base + _NSEM * blk, blk, t + 1 + _NSEM, sem):
                c.start()

        @pl.when(t == ramp_out_step)
        def _():
            sl = pl.ds(0, ramp)
            pltpu.make_async_copy(ob.at[sl], o_hbm.at[sl], sem_out.at[0]).start()

        emit(main_ops, main_items, base, t + 1, (0, 1, 2), None, True)
        return carry

    def everything(_, carry):
        emit(ramp_ops, ramp_items, 0, 0, (), ramp_fence, False)
        return jax.lax.fori_loop(0, nblk, main_block, carry)

    for g in range(_NSEM):
        start_group(g)

    one_ref[0] = 1
    jax.lax.fori_loop(0, one_ref[0], everything, 0)

    pltpu.make_async_copy(ob, o_hbm, sem_out.at[0]).wait()


@jax.jit
def pallas_standalone__gqa_softmax__near_ridge_kernel(q, k, v):
    B, Hq, Sq, D = q.shape
    Hkv, Sk = k.shape[1], k.shape[2]
    rep = Hq // Hkv
    G, rows = B * Hkv, rep * Sq
    ramp_sizes, blk, nblk = (1, 2, 4), 8, 7
    assert 1 + sum(ramp_sizes) + blk * nblk == G
    assert rows % _TQ == 0 and rows >= 8 * _TQ and Sk > _KT

    out = pl.pallas_call(
        functools.partial(_attn_kernel, scale=float(D) ** -0.5, ramp_sizes=ramp_sizes,
                          nfirst=4, blk=blk, nblk=nblk, ramp_out_step=3),
        in_specs=[pl.BlockSpec(memory_space=pl.ANY)] * 3,
        out_specs=pl.BlockSpec(memory_space=pl.ANY),
        out_shape=jax.ShapeDtypeStruct((G, rows, D), q.dtype),
        scratch_shapes=[
            pltpu.VMEM((G, rows, D), q.dtype),
            pltpu.VMEM((G, Sk, D), k.dtype),
            pltpu.VMEM((G, Sk, D), v.dtype),
            pltpu.VMEM((G, rows, D), q.dtype),
            pltpu.VMEM((nblk + 1, _KT, D), k.dtype),
            pltpu.VMEM((D, _KT), k.dtype),
            pltpu.SemaphoreType.DMA((_NSEM,)),
            pltpu.SemaphoreType.DMA((1,)),
            pltpu.SMEM((1,), jnp.int32),
        ],
        compiler_params=pltpu.CompilerParams(
            vmem_limit_bytes=120 * 1024 * 1024,
            disable_bounds_checks=True,
        ),
    )(q.reshape(G, rows, D), k.reshape(G, Sk, D), v.reshape(G, Sk, D))
    return out.reshape(B, Hq, Sq, D)
```

```python
import functools

import jax
import jax.numpy as jnp
import jax.experimental.pallas as pl
import jax.experimental.pallas.tpu as pltpu

_LOG2E = 1.4426950408889634
_TQ = 128
_DEPTH = 2
_NSEM = 2
_KT = 256
_LAST_SPLIT = 4
_NT = (((1,), (1,)), ((), ()))


def _make_items(ngroups, rows, first_chunks=()):
    items, off = [], 0
    for c in first_chunks:
        items.append((0, off, c))
        off += c
    while off < rows:
        items.append((0, off, _TQ))
        off += _TQ
    for g in range(1, ngroups):
        for c in range(rows // _TQ):
            items.append((g, c * _TQ, _TQ))
    return items


def _block_ops(n):
    ops, nq, npv = [], 0, 0
    while npv < n:
        if nq < n and nq - npv <= _DEPTH:
            ops.append(("q", nq))
            nq += 1
        else:
            ops += [("s", npv), ("p", npv)]
            npv += 1
    return ops


def _ramp_ops(items, ramp_sizes, nfirst):
    n = len(items)
    firsts, acc = [], 1
    for sz in ramp_sizes:
        firsts.append(acc)
        acc += sz
    bounds = [j for j, it in enumerate(items) if it[0] in firsts and it[1] == 0]
    mxu = [("f", 0)] + [("q", j) for j in range(nfirst)] + [("f", 1)]
    nq, npv, g = nfirst, 0, 2
    while npv < n:
        if nq < n and nq - npv <= _DEPTH:
            mxu.append(("q", nq))
            nq += 1
        else:
            if nq in bounds and nq - npv == _DEPTH + 1:
                mxu.append(("f", g))
                g += 1
                bounds.remove(nq)
            mxu.append(("p", npv))
            npv += 1
    ops, ns, nq = [], 0, 0
    for op, j in mxu:
        upto = {"f": nq - 1, "p": j + 1, "q": 0}[op]
        while ns < upto:
            ops.append(("s", ns))
            ns += 1
        nq += op == "q"
        ops.append((op, j))
    return ops


def _attn_kernel(q_hbm, k_hbm, v_hbm, o_hbm, qb, kb, vb, ob, kf, kt,
                 sem_in, sem_out, *,
                 scale, ramp_sizes, nfirst, blk, nblk, ramp_out_step):
    ngroups, rows = qb.shape[0], qb.shape[1]
    ramp = 1 + sum(ramp_sizes)
    ramp_items = _make_items(ramp, rows)
    main_items = _make_items(blk, rows, (_TQ, _TQ, 2 * _TQ))
    first_rows = nfirst * _TQ

    def group_copies(g0, n, kf_slot, sem):
        sl = pl.ds(g0, n)
        cps = [pltpu.make_async_copy(k_hbm.at[sl], kb.at[sl], sem),
               pltpu.make_async_copy(q_hbm.at[sl], qb.at[sl], sem),
               pltpu.make_async_copy(v_hbm.at[sl], vb.at[sl], sem)]
        if kf_slot is not None:
            nxt = jnp.minimum(g0 + n, ngroups - 1)
            cps.append(pltpu.make_async_copy(
                k_hbm.at[nxt, pl.ds(0, _KT)], kf.at[kf_slot], sem))
        return cps

    def first_copies(sem):
        sl = pl.ds(0, first_rows)
        return [pltpu.make_async_copy(k_hbm.at[0], kb.at[0], sem),
                pltpu.make_async_copy(q_hbm.at[0, sl], qb.at[0, sl], sem)]

    def second_copies(sem):
        sl = pl.ds(first_rows, rows - first_rows)
        return [pltpu.make_async_copy(v_hbm.at[0], vb.at[0], sem),
                pltpu.make_async_copy(q_hbm.at[0, sl], qb.at[0, sl], sem)]

    dma_groups = [first_copies, second_copies]
    g0 = 1
    for i, sz in enumerate(ramp_sizes):
        slot = 0 if i == len(ramp_sizes) - 1 else None
        dma_groups.append(functools.partial(group_copies, g0, sz, slot))
        g0 += sz
    n_ramp_dma = len(dma_groups)
    for t in range(nblk):
        dma_groups.append(functools.partial(group_copies, ramp + t * blk, blk, t + 1))

    def start_group(g):
        for c in dma_groups[g](sem_in.at[g % _NSEM]):
            c.start()

    def out_copy(g, r0, n):
        sl = pl.ds(r0, n)
        return pltpu.make_async_copy(ob.at[g, sl], o_hbm.at[g, sl], sem_out.at[0])

    def emit(ops, items, base, kf_slot, exp2_items, fence, main):
        scores, probs = {}, {}
        last_group = items[-1][0]
        for idx, (op, j) in enumerate(ops):
            if idx == len(ops) - 20:
                kt[...] = kf[kf_slot].T
            if op == "f":
                fence(j)
                continue
            gl, r0, n = items[j]
            g = base + gl
            if op == "q":
                qv = qb[g, pl.ds(r0, n), :]
                if main and j == 0:
                    s0 = jnp.dot(qv, kt[...], preferred_element_type=jnp.float32)
                    s1 = jax.lax.dot_general(
                        qv, kb[g, pl.ds(_KT, kb.shape[1] - _KT), :], _NT,
                        preferred_element_type=jnp.float32)
                    scores[j] = jnp.concatenate([s0, s1], axis=1)
                else:
                    scores[j] = jax.lax.dot_general(
                        qv, kb[g], _NT, preferred_element_type=jnp.float32)
            elif op == "s":
                s = scores.pop(j)
                m = jnp.max(s, axis=-1, keepdims=True)
                if j in exp2_items:
                    p = jnp.exp2((s - m) * (scale * _LOG2E))
                else:
                    p = jnp.exp((s - m) * scale)
                l = jnp.sum(p, axis=-1, keepdims=True)
                r = pl.reciprocal(l, approx=True)
                r = r * (2.0 - l * r)
                probs[j] = (p * r).astype(vb.dtype)
            else:
                o = jnp.dot(probs.pop(j), vb[g],
                            preferred_element_type=jnp.float32).astype(ob.dtype)
                if main and j == len(items) - 1:
                    per = n // _LAST_SPLIT
                    for u in range(_LAST_SPLIT):
                        ob[g, pl.ds(r0 + u * per, per), :] = o[u * per:(u + 1) * per]
                        out_copy(g, r0 + u * per, per).start()
                    continue
                ob[g, pl.ds(r0, n), :] = o
                if main and gl == last_group:
                    out_copy(g, r0, n).start()
                elif main and r0 + n == rows:
                    out_copy(g, 0, rows).start()

    def ramp_fence(g):
        for c in dma_groups[g](sem_in.at[g % _NSEM]):
            c.wait()
        start_group(g + _NSEM)

    ramp_ops = _ramp_ops(ramp_items, ramp_sizes, nfirst)
    main_ops = _block_ops(len(main_items))

    def main_block(t, carry):
        base = ramp + t * blk
        sem = sem_in.at[(n_ramp_dma + t) % _NSEM]
        for c in group_copies(base, blk, t + 1, sem):
            c.wait()

        @pl.when(t + _NSEM < nblk)
        def _():
            for c in group_copies(base + _NSEM * blk, blk, t + 1 + _NSEM, sem):
                c.start()

        @pl.when(t == ramp_out_step)
        def _():
            sl = pl.ds(0, ramp)
            pltpu.make_async_copy(ob.at[sl], o_hbm.at[sl], sem_out.at[0]).start()

        emit(main_ops, main_items, base, t + 1, (0, 1, 2), None, True)
        return carry

    @pl.when(pl.program_id(0) == 0)
    def _():
        for g in range(_NSEM):
            start_group(g)
        emit(ramp_ops, ramp_items, 0, 0, (), ramp_fence, False)

    @pl.when(pl.program_id(0) == 1)
    def _():
        jax.lax.fori_loop(0, nblk, main_block, 0)
        pltpu.make_async_copy(ob, o_hbm, sem_out.at[0]).wait()


@jax.jit
def pallas_standalone__gqa_softmax__near_ridge_kernel(q, k, v):
    B, Hq, Sq, D = q.shape
    Hkv, Sk = k.shape[1], k.shape[2]
    rep = Hq // Hkv
    G, rows = B * Hkv, rep * Sq
    ramp_sizes, blk, nblk = (1, 2, 4), 8, 7
    assert 1 + sum(ramp_sizes) + blk * nblk == G
    assert rows % _TQ == 0 and rows >= 8 * _TQ and Sk > _KT

    out = pl.pallas_call(
        functools.partial(_attn_kernel, scale=float(D) ** -0.5, ramp_sizes=ramp_sizes,
                          nfirst=4, blk=blk, nblk=nblk, ramp_out_step=3),
        grid=(2,),
        in_specs=[pl.BlockSpec(memory_space=pl.ANY)] * 3,
        out_specs=pl.BlockSpec(memory_space=pl.ANY),
        out_shape=jax.ShapeDtypeStruct((G, rows, D), q.dtype),
        scratch_shapes=[
            pltpu.VMEM((G, rows, D), q.dtype),
            pltpu.VMEM((G, Sk, D), k.dtype),
            pltpu.VMEM((G, Sk, D), v.dtype),
            pltpu.VMEM((G, rows, D), q.dtype),
            pltpu.VMEM((nblk + 1, _KT, D), k.dtype),
            pltpu.VMEM((D, _KT), k.dtype),
            pltpu.SemaphoreType.DMA((_NSEM,)),
            pltpu.SemaphoreType.DMA((1,)),
        ],
        compiler_params=pltpu.CompilerParams(
            dimension_semantics=("arbitrary",),
            vmem_limit_bytes=120 * 1024 * 1024,
            disable_bounds_checks=True,
        ),
    )(q.reshape(G, rows, D), k.reshape(G, Sk, D), v.reshape(G, Sk, D))
    return out.reshape(B, Hq, Sq, D)
```
